```python
import jax
import jax.numpy as jnp

def _softmax(x, axis=-1):
    return jax.nn.softmax(x, axis=axis)
def _gelu(x):
    return jax.nn.gelu(x, approximate=True)
def _silu(x):
    return jax.nn.silu(x)
def _sigmoid(x):
    return jax.nn.sigmoid(x)
def _layernorm(x, axis=-1, eps=1e-5):
    m = jnp.mean(x, axis=axis, keepdims=True)
    v = jnp.var(x, axis=axis, keepdims=True)
    return (x - m) / jnp.sqrt(v + eps)
def _scatter_add(tgt, idx, src, axis=0):
    return tgt.at[idx].add(src)
def _segment_sum(src, seg, n):
    return jax.ops.segment_sum(src, seg, n)
class _Rng:
    def __init__(self, key):
        self._k = key
    def _next(self):
        self._k, sub = jax.random.split(self._k)
        return sub
    def normal(self, shape):
        return jax.random.normal(self._next(), shape, dtype=jnp.bfloat16)
    def randint(self, lo, hi, shape):
        return jax.random.randint(self._next(), shape, lo, hi, dtype=jnp.int32)
    def uniform(self, shape, lo=0.0, hi=1.0):
        return jax.random.uniform(self._next(), shape, jnp.bfloat16, lo, hi)
    def permutation(self, n):
        return jax.random.permutation(self._next(), n)


kernel_name = 'recurrent_scan__sliding_block_cached__moe_arch_mod__decode'

def setup_inputs():
    _rng = _Rng(jax.random.key(int.from_bytes(__import__("os").urandom(4), "little")))
    _w = (lambda a: (lambda t: t.astype(jnp.bfloat16) if jnp.issubdtype(t.dtype, jnp.floating) else t)(jnp.asarray(a)))
    def _A_setup():
        B, Sq, D = 1, 1, 512
        Hq, Hkv, Sk, Dh = 32, 32, 32768, 128
        assert Hq % Hkv == 0, (Hq, Hkv)
        return {
            "x": _w((lambda *s: _rng.normal(s) * 0.05)(B, Sq, D)),
            "k_cache": _w((lambda *s: _rng.normal(s) * 0.05)(B, Hkv, Sk, Dh)),
            "v_cache": _w((lambda *s: _rng.normal(s) * 0.05)(B, Hkv, Sk, Dh)),
            "wq": _w((lambda *s: _rng.normal(s) * 0.05)(D, Hq * Dh) * (D ** -0.5)),
            "wo": _w((lambda *s: _rng.normal(s) * 0.05)(Hq * Dh, D) * ((Hq * Dh) ** -0.5)),
        }
    _A_in = _A_setup()

    def _B_setup():
        B, S, D, F, C = 1, 1, 512, 1376, 1
        return {
            "x": _w((lambda *s: _rng.normal(s) * 0.05)(B, S, D)),
            "w_r": _w((lambda *s: _rng.normal(s) * 0.05)(D)),
            "w_gate": _w((lambda *s: _rng.normal(s) * 0.05)(D, F)),
            "w_up": _w((lambda *s: _rng.normal(s) * 0.05)(D, F)),
            "w_down": _w((lambda *s: _rng.normal(s) * 0.05)(F, D)),
        }
    _B_in = _B_setup()

    return {
        "A_x": _A_in["x"],
        "A_k_cache": _A_in["k_cache"],
        "A_v_cache": _A_in["v_cache"],
        "A_wq": _A_in["wq"],
        "A_wo": _A_in["wo"],
        "B_x": _B_in["x"],
        "B_w_r": _B_in["w_r"],
        "B_w_gate": _B_in["w_gate"],
        "B_w_up": _B_in["w_up"],
        "B_w_down": _B_in["w_down"],
    }

def reference(A_x, A_k_cache, A_v_cache, A_wq, A_wo, B_x, B_w_r, B_w_gate, B_w_up, B_w_down):
    def _A_ref(x, k_cache, v_cache, wq, wo):
        B, Sq, D = x.shape
        Hq, Dh = 32, 128
        Hkv, Sk = k_cache.shape[1], k_cache.shape[2]
        W = min(4096, max(256, Sk // 4))
        rep = Hq // Hkv
        q = (lambda x, *d: x.transpose(*d))((x @ wq).reshape(B, Sq, Hq, Dh), 0, 2, 1, 3)
        k = jnp.repeat(k_cache[:, :, Sk - W:, :], rep, axis=1)
        v = jnp.repeat(v_cache[:, :, Sk - W:, :], rep, axis=1)
        scores = jnp.einsum("bhqd,bhkd->bhqk", q, k) * (Dh ** -0.5)
        p = _softmax(scores, axis=-1)
        o = jnp.einsum("bhqk,bhkd->bhqd", p, v)
        return (lambda x, *d: x.transpose(*d))(o, 0, 2, 1, 3).reshape(B, Sq, Hq * Dh) @ wo

    def _B_ref(x, w_r, w_gate, w_up, w_down):
        B, S, D = x.shape
        C = 1
        r = x @ w_r
        idx = jnp.argsort(-r, axis=-1)[:, :C]
        idx_e = jnp.repeat(idx.reshape(B, C, 1), D, axis=2)
        x_sel = jnp.take_along_axis(x, idx_e, axis=1)
        g = _silu(x_sel @ w_gate)
        u = x_sel @ w_up
        y = (g * u) @ w_down
        r_sel = _sigmoid(jnp.take_along_axis(r, idx, axis=1))
        y = y * r_sel.reshape(B, C, 1)
        b_off = (jnp.arange(B) * S).reshape(B, 1)
        flat_idx = (idx + b_off).reshape(B * C)
        zero = (x * 0.0).reshape(B * S, D)
        upd = _scatter_add(zero, flat_idx, y.reshape(B * C, D), axis=0)
        return x + upd.reshape(B, S, D)

    x = A_x
    xn = _layernorm(x, axis=-1)
    s = _A_ref(xn, A_k_cache, A_v_cache, A_wq, A_wo)
    g = _silu(_B_ref(xn, B_w_r, B_w_gate, B_w_up, B_w_down))
    return x + s * g
```

```python
import jax
import jax.numpy as jnp
import numpy as np
import jax.experimental.pallas as pl
import jax.experimental.pallas.tpu as pltpu

_HQ, _DH = 32, 128
_M = 8
_WO_MXU_CHUNKS = (2048, 1024, 512, 256, 128)
_WO_VPU_CHUNKS = (64, 64)

_NT = (((1,), (1,)), ((), ()))


def _sigmoid(x):
    return jax.nn.sigmoid(x)


@jax.jit
def pallas_recurrent_scan__sliding_block_cached__moe_arch_mod__decode_kernel(
    A_x: jax.Array,
    A_k_cache: jax.Array,
    A_v_cache: jax.Array,
    A_wq: jax.Array,
    A_wo: jax.Array,
    B_x: jax.Array,
    B_w_r: jax.Array,
    B_w_gate: jax.Array,
    B_w_up: jax.Array,
    B_w_down: jax.Array,
):
    del B_x
    H, DH, M = _HQ, _DH, _M
    D = A_x.shape[-1]
    F = B_w_gate.shape[1]
    Sk = A_k_cache.shape[2]
    W = min(4096, max(256, Sk // 4))
    assert A_x.shape == (1, 1, D) and A_k_cache.shape[1] == H

    chunks = _WO_MXU_CHUNKS + _WO_VPU_CHUNKS
    n_mxu, n_wo = len(_WO_MXU_CHUNKS), len(chunks)
    wo_off = np.concatenate([[0], np.cumsum(chunks)]).tolist()
    assert wo_off[-1] == H * DH and wo_off[n_mxu] >= (H - 1) * DH

    S_X, S_WR, S_WQ, S_G, S_U, S_D, S_K = range(7)
    S_V = S_K + H
    S_WO = S_V + H
    n_sem = S_WO + n_wo
    f32, bf16 = jnp.float32, jnp.bfloat16
    scale = DH ** -0.5

    def kernel(x_hbm, k_hbm, v_hbm, wq_hbm, wo_hbm, wr_hbm, wg_hbm, wu_hbm, wd_hbm,
               o_ref,
               x_v, wr_v, wq_v, wg_v, wu_v, wd_v, wo_v, k_v, v_v, q_s, o_s, sems):
        cx = pltpu.make_async_copy(x_hbm, x_v, sems.at[S_X])
        cwr = pltpu.make_async_copy(wr_hbm, wr_v, sems.at[S_WR])
        cwq = pltpu.make_async_copy(wq_hbm, wq_v, sems.at[S_WQ])
        cg = pltpu.make_async_copy(wg_hbm, wg_v, sems.at[S_G])
        cu = pltpu.make_async_copy(wu_hbm, wu_v, sems.at[S_U])
        cd = pltpu.make_async_copy(wd_hbm, wd_v, sems.at[S_D])

        def ck(h):
            return pltpu.make_async_copy(
                k_hbm.at[0, h, pl.ds(Sk - W, W), :], k_v.at[h], sems.at[S_K + h])

        def cv(h):
            return pltpu.make_async_copy(
                v_hbm.at[0, h, pl.ds(Sk - W, W), :], v_v.at[h], sems.at[S_V + h])

        def cwo(i):
            rows = pl.ds(wo_off[i], chunks[i])
            return pltpu.make_async_copy(
                wo_hbm.at[rows, :], wo_v.at[rows, :], sems.at[S_WO + i])

        cwq.start()
        cx.start()
        cwr.start()
        for h in range(H):
            ck(h).start()
            cv(h).start()
        cg.start()
        cu.start()
        cd.start()
        for i in range(n_wo):
            cwo(i).start()

        cx.wait()
        x = x_v[0].astype(f32)
        mu = jnp.mean(x, axis=-1, keepdims=True)
        xc = x - mu
        var = jnp.mean(xc * xc, axis=-1, keepdims=True)
        xn = (xc / jnp.sqrt(var + 1e-5)).astype(bf16)
        xn_m = jnp.broadcast_to(xn, (M, D))

        cwq.wait()
        q = jnp.dot(xn_m, wq_v[...], preferred_element_type=f32).astype(bf16)
        for h in range(H):
            q_s[h] = q[:, h * DH:(h + 1) * DH]

        def head(h, carry):
            ck(h).wait()
            s = jax.lax.dot_general(q_s[h], k_v[h], _NT, preferred_element_type=f32)
            s = s * scale
            m = jnp.max(s, axis=-1, keepdims=True)
            p = jnp.exp(s - m)
            l = jnp.sum(p, axis=-1, keepdims=True)
            pb = p.astype(bf16)
            cv(h).wait()
            o = jnp.dot(pb, v_v[h], preferred_element_type=f32)
            o_s[h] = (o / l).astype(bf16)
            return carry

        jax.lax.fori_loop(0, H, head, 0)

        orow = o_s[H - 1].astype(f32)[0:1]
        ocol = jnp.transpose(jnp.broadcast_to(orow, (DH, DH)))

        cwr.wait()
        xnf = xn.astype(f32)
        wr = wr_v[...].astype(f32).reshape(1, D)
        r = jnp.sum(xnf * wr, axis=-1, keepdims=True)
        cg.wait()
        gt = jax.lax.dot_general(xn_m, wg_v[...], _NT, preferred_element_type=f32)
        cu.wait()
        up = jax.lax.dot_general(xn_m, wu_v[...], _NT, preferred_element_type=f32)
        gt = gt.astype(bf16).astype(f32)
        up = up.astype(bf16).astype(f32)
        hh = (gt * _sigmoid(gt) * up).astype(bf16)
        cd.wait()
        y = jnp.dot(hh, wd_v[...], preferred_element_type=f32)[0:1]
        y = y * _sigmoid(r)
        b = xnf + (xnf * 0.0 + y)
        gate = b * _sigmoid(b)

        acc = jnp.zeros((M, D), f32)
        for i in range(n_mxu):
            a, e = wo_off[i], wo_off[i + 1]
            oc = jnp.concatenate([o_s[h] for h in range(a // DH, e // DH)], axis=1)
            cwo(i).wait()
            acc = acc + jnp.dot(oc, wo_v[a:e, :], preferred_element_type=f32)
        base = x + acc[0:1] * gate
        part = jnp.zeros((8, D), f32)
        for i in range(n_mxu, n_wo):
            a, e = wo_off[i], wo_off[i + 1]
            oc = ocol[a - (H - 1) * DH:e - (H - 1) * DH]
            cwo(i).wait()
            w = wo_v[a:e, :].astype(f32)
            prod = w * jnp.concatenate([oc] * (D // DH), axis=1)
            part = part + jnp.sum(prod.reshape((e - a) // 8, 8, D), axis=0)
        out = base + jnp.sum(part, axis=0, keepdims=True) * gate
        o_ref[0] = out.astype(o_ref.dtype)

    hbm = pl.BlockSpec(memory_space=pltpu.HBM)
    return pl.pallas_call(
        kernel,
        out_shape=jax.ShapeDtypeStruct(A_x.shape, A_x.dtype),
        in_specs=[hbm] * 9,
        out_specs=pl.BlockSpec(memory_space=pltpu.VMEM),
        scratch_shapes=[
            pltpu.VMEM((1, 1, D), bf16),
            pltpu.VMEM((D,), bf16),
            pltpu.VMEM((D, H * DH), bf16),
            pltpu.VMEM((F, D), bf16),
            pltpu.VMEM((F, D), bf16),
            pltpu.VMEM((F, D), bf16),
            pltpu.VMEM((H * DH, D), bf16),
            pltpu.VMEM((H, W, DH), bf16),
            pltpu.VMEM((H, W, DH), bf16),
            pltpu.VMEM((H, M, DH), bf16),
            pltpu.VMEM((H, M, DH), bf16),
            pltpu.SemaphoreType.DMA((n_sem,)),
        ],
        compiler_params=pltpu.CompilerParams(
            vmem_limit_bytes=110 * 2**20,
            disable_semaphore_checks=True,
        ),
    )(A_x, A_k_cache, A_v_cache, A_wq, A_wo, B_w_r, B_w_gate.T, B_w_up.T, B_w_down)
```

```python
import jax
import jax.numpy as jnp
import numpy as np
import jax.experimental.pallas as pl
import jax.experimental.pallas.tpu as pltpu

_HQ, _DH = 32, 128
_M = 8
_KV_ROWS = 192
_W_ROWS = 48
_WQ_TILE = (24, 1024)
_LOOKAHEAD = 3
_N_TAIL = 4
_WO_MXU = (2048, 1024, 512)
_WO_VPU = (256, 128, 64, 32, 32)

_NT = (((1,), (1,)), ((), ()))


def _split(n, c, start=0):
    return [(start + p, min(c, n - p)) for p in range(0, n, c)]


@jax.jit
def pallas_recurrent_scan__sliding_block_cached__moe_arch_mod__decode_kernel(
    A_x: jax.Array,
    A_k_cache: jax.Array,
    A_v_cache: jax.Array,
    A_wq: jax.Array,
    A_wo: jax.Array,
    B_x: jax.Array,
    B_w_r: jax.Array,
    B_w_gate: jax.Array,
    B_w_up: jax.Array,
    B_w_down: jax.Array,
):
    del B_x
    H, DH, M, L = _HQ, _DH, _M, _LOOKAHEAD
    D = A_x.shape[-1]
    F = B_w_gate.shape[1]
    Sk = A_k_cache.shape[2]
    W = min(4096, max(256, Sk // 4))
    assert A_x.shape == (1, 1, D) and A_k_cache.shape[1] == H

    chunks = _WO_MXU + _WO_VPU
    n_mxu, n_wo = len(_WO_MXU), len(chunks)
    wo_off = np.concatenate([[0], np.cumsum(chunks)]).tolist()
    assert wo_off[-1] == H * DH and wo_off[n_mxu] % DH == 0
    hv0 = wo_off[n_mxu] // DH

    S_X, S_WR, S_WQ, S_G, S_U, S_D, S_K = range(7)
    S_V = S_K + H
    S_WO = S_V + H
    n_sem = S_WO + n_wo
    f32, bf16 = jnp.float32, jnp.bfloat16
    scale = DH ** -0.5

    def kernel(x_hbm, k_hbm, v_hbm, wq_hbm, wo_hbm, wr_hbm, wg_hbm, wu_hbm, wd_hbm,
               o_ref,
               x_v, wr_v, wq_v, wg_v, wu_v, wd_v, wo_v, k_v, v_v, q_s, o_s, sems):
        mk = pltpu.make_async_copy

        def wait_all(buf, sem):
            mk(buf, buf, sem).wait()

        def row_copies(hbm, vm, sem, n, start=0):
            return [mk(hbm.at[pl.ds(p, r), :], vm.at[pl.ds(p, r), :], sems.at[sem])
                    for p, r in _split(n, _W_ROWS, start)]

        def start_alternating(copies, first=0):
            for j, c in enumerate(copies):
                c.start(priority=(first + j) % 2)

        cx = mk(x_hbm, x_v, sems.at[S_X])
        cwr = mk(wr_hbm, wr_v, sems.at[S_WR])
        wq_copies = [
            mk(wq_hbm.at[pl.ds(p, r), pl.ds(c0, cw)],
               wq_v.at[pl.ds(p, r), pl.ds(c0, cw)], sems.at[S_WQ])
            for p, r in _split(D, _WQ_TILE[0])
            for c0, cw in _split(H * DH, _WQ_TILE[1])]
        tail = (row_copies(wg_hbm, wg_v, S_G, F) + row_copies(wu_hbm, wu_v, S_U, F)
                + row_copies(wd_hbm, wd_v, S_D, F))
        for i in range(n_wo):
            tail += row_copies(wo_hbm, wo_v, S_WO + i, chunks[i], wo_off[i])
        cuts = [round(j * len(tail) / _N_TAIL) for j in range(_N_TAIL + 1)]

        def issue_tail(j):
            start_alternating(tail[cuts[j]:cuts[j + 1]], cuts[j])

        def issue_head(h):
            for p, r in _split(W, _KV_ROWS):
                mk(k_hbm.at[0, h, pl.ds(Sk - W + p, r), :], k_v.at[h, pl.ds(p, r), :],
                   sems.at[S_K + h]).start(priority=0)
                mk(v_hbm.at[0, h, pl.ds(Sk - W + p, r), :], v_v.at[h, pl.ds(p, r), :],
                   sems.at[S_V + h]).start(priority=1)

        cx.start()
        cwr.start()
        start_alternating(wq_copies)
        for h in range(L):
            issue_head(h)

        cx.wait()
        x = x_v[0].astype(f32)
        mu = jnp.mean(x, axis=-1, keepdims=True)
        xc = x - mu
        var = jnp.mean(xc * xc, axis=-1, keepdims=True)
        xn = (xc / jnp.sqrt(var + 1e-5)).astype(bf16)
        xn_m = jnp.broadcast_to(xn, (M, D))

        wait_all(wq_v, sems.at[S_WQ])
        q = jnp.dot(xn_m, wq_v[...], preferred_element_type=f32).astype(bf16)
        for h in range(H):
            q_s[h] = q[:, h * DH:(h + 1) * DH]

        def head(h, carry):
            nxt = h + L

            @pl.when(nxt < H)
            def _():
                issue_head(nxt)

            for j in range(min(L, _N_TAIL)):
                @pl.when(nxt == H + j)
                def _():
                    issue_tail(j)

            wait_all(k_v.at[h], sems.at[S_K + h])
            s = jax.lax.dot_general(q_s[h], k_v[h], _NT, preferred_element_type=f32)
            s = s * scale
            m = jnp.max(s, axis=-1, keepdims=True)
            p = jnp.exp(s - m)
            l = jnp.sum(p, axis=-1, keepdims=True)
            pb = p.astype(bf16)
            wait_all(v_v.at[h], sems.at[S_V + h])
            o = jnp.dot(pb, v_v[h], preferred_element_type=f32)
            o_s[h] = (o / l).astype(bf16)
            return carry

        jax.lax.fori_loop(0, H, head, 0)
        for j in range(min(L, _N_TAIL), _N_TAIL):
            issue_tail(j)

        ocol = jnp.concatenate([
            jnp.transpose(jnp.broadcast_to(o_s[h].astype(f32)[0:1], (DH, DH)))
            for h in range(hv0, H)], axis=0)

        cwr.wait()
        xnf = xn.astype(f32)
        wr = wr_v[...].astype(f32).reshape(1, D)
        r = jnp.sum(xnf * wr, axis=-1, keepdims=True)
        wait_all(wg_v, sems.at[S_G])
        gt = jax.lax.dot_general(xn_m, wg_v[...], _NT, preferred_element_type=f32)
        wait_all(wu_v, sems.at[S_U])
        up = jax.lax.dot_general(xn_m, wu_v[...], _NT, preferred_element_type=f32)
        gt = gt.astype(bf16).astype(f32)
        up = up.astype(bf16).astype(f32)
        hh = (gt * jax.nn.sigmoid(gt) * up).astype(bf16)
        wait_all(wd_v, sems.at[S_D])
        y = jnp.dot(hh, wd_v[...], preferred_element_type=f32)[0:1]
        y = y * jax.nn.sigmoid(r)
        b = xnf + (xnf * 0.0 + y)
        gate = b * jax.nn.sigmoid(b)

        acc = jnp.zeros((M, D), f32)
        for i in range(n_mxu):
            a, e = wo_off[i], wo_off[i + 1]
            oc = jnp.concatenate([o_s[h] for h in range(a // DH, e // DH)], axis=1)
            wait_all(wo_v.at[pl.ds(a, e - a), :], sems.at[S_WO + i])
            acc = acc + jnp.dot(oc, wo_v[a:e, :], preferred_element_type=f32)
        base = x + acc[0:1] * gate
        part = jnp.zeros((8, D), f32)
        for i in range(n_mxu, n_wo):
            a, e = wo_off[i], wo_off[i + 1]
            oc = ocol[a - hv0 * DH:e - hv0 * DH]
            wait_all(wo_v.at[pl.ds(a, e - a), :], sems.at[S_WO + i])
            w = wo_v[a:e, :].astype(f32)
            prod = w * jnp.concatenate([oc] * (D // DH), axis=1)
            part = part + jnp.sum(prod.reshape((e - a) // 8, 8, D), axis=0)
        out = base + jnp.sum(part, axis=0, keepdims=True) * gate
        o_ref[0] = out.astype(o_ref.dtype)

    hbm = pl.BlockSpec(memory_space=pltpu.HBM)
    return pl.pallas_call(
        kernel,
        out_shape=jax.ShapeDtypeStruct(A_x.shape, A_x.dtype),
        in_specs=[hbm] * 9,
        out_specs=pl.BlockSpec(memory_space=pltpu.VMEM),
        scratch_shapes=[
            pltpu.VMEM((1, 1, D), bf16),
            pltpu.VMEM((D,), bf16),
            pltpu.VMEM((D, H * DH), bf16),
            pltpu.VMEM((F, D), bf16),
            pltpu.VMEM((F, D), bf16),
            pltpu.VMEM((F, D), bf16),
            pltpu.VMEM((H * DH, D), bf16),
            pltpu.VMEM((H, W, DH), bf16),
            pltpu.VMEM((H, W, DH), bf16),
            pltpu.VMEM((H, M, DH), bf16),
            pltpu.VMEM((H, M, DH), bf16),
            pltpu.SemaphoreType.DMA((n_sem,)),
        ],
        compiler_params=pltpu.CompilerParams(
            vmem_limit_bytes=110 * 2**20,
            disable_semaphore_checks=True,
        ),
    )(A_x, A_k_cache, A_v_cache, A_wq, A_wo, B_w_r, B_w_gate.T, B_w_up.T, B_w_down)
```

```python
import jax
import jax.numpy as jnp
import numpy as np
import jax.experimental.pallas as pl
import jax.experimental.pallas.tpu as pltpu

_HQ, _DH = 32, 128
_M = 8
_KV_ROWS = 188
_W_ROWS = 40
_WQ_TILE = (8, 2560)
_PRIME = 26
_LOOKAHEAD = 3
_N_TAIL = 4
_WO_GROUP = 512
_WO_MXU = (_WO_GROUP,) * 7
_WO_VPU = (256, 128, 64, 32, 32)

_NT = (((1,), (1,)), ((), ()))


def _split(n, c, start=0):
    return [(start + p, min(c, n - p)) for p in range(0, n, c)]


@jax.jit
def pallas_recurrent_scan__sliding_block_cached__moe_arch_mod__decode_kernel(
    A_x: jax.Array,
    A_k_cache: jax.Array,
    A_v_cache: jax.Array,
    A_wq: jax.Array,
    A_wo: jax.Array,
    B_x: jax.Array,
    B_w_r: jax.Array,
    B_w_gate: jax.Array,
    B_w_up: jax.Array,
    B_w_down: jax.Array,
):
    del B_x
    H, DH, M, L = _HQ, _DH, _M, _LOOKAHEAD
    D = A_x.shape[-1]
    F = B_w_gate.shape[1]
    Sk = A_k_cache.shape[2]
    W = min(4096, max(256, Sk // 4))
    assert A_x.shape == (1, 1, D) and A_k_cache.shape[1] == H

    chunks = _WO_MXU + _WO_VPU
    n_mxu, n_wo = len(_WO_MXU), len(chunks)
    wo_off = np.concatenate([[0], np.cumsum(chunks)]).tolist()
    assert wo_off[-1] == H * DH and wo_off[n_mxu] % DH == 0
    hv0 = wo_off[n_mxu] // DH

    S_X, S_WR, S_WQ, S_G, S_U, S_D, S_K = range(7)
    S_V = S_K + H
    S_WO = S_V + H
    n_sem = S_WO + n_wo
    f32, bf16 = jnp.float32, jnp.bfloat16
    scale = DH ** -0.5

    def kernel(x_hbm, k_hbm, v_hbm, wq_hbm, wo_hbm, wr_hbm, wg_hbm, wu_hbm, wd_hbm,
               o_ref,
               x_v, wr_v, wq_v, wg_v, wu_v, wd_v, wo_v, k_v, v_v, q_s, o_s, sems):
        mk = pltpu.make_async_copy

        def wait_all(buf, sem):
            mk(buf, buf, sem).wait()

        def row_copies(hbm, vm, sem, n, start=0):
            return [(mk(hbm.at[pl.ds(p, r), :], vm.at[pl.ds(p, r), :], sems.at[sem]), r)
                    for p, r in _split(n, _W_ROWS, start)]

        def wq_copies(r0, r1):
            return [(mk(wq_hbm.at[pl.ds(p, r), pl.ds(c0, cw)],
                        wq_v.at[pl.ds(p, r), pl.ds(c0, cw)], sems.at[S_WQ]), r * cw)
                    for p, r in _split(r1 - r0, _WQ_TILE[0], r0)
                    for c0, cw in _split(H * DH, _WQ_TILE[1])]

        def merge(a, b, prime=0):
            out = [(c, 1) for c, _ in b[:prime]]
            ia, ib, na, nb = 0, min(prime, len(b)), 0, 0
            while ia < len(a) or ib < len(b):
                if ia < len(a) and (ib >= len(b) or na <= nb):
                    out.append((a[ia][0], 0))
                    na += a[ia][1]
                    ia += 1
                else:
                    out.append((b[ib][0], 1))
                    nb += b[ib][1]
                    ib += 1
            return out

        def start_all(copies):
            for c, prio in copies:
                c.start(priority=prio)

        cx = mk(x_hbm, x_v, sems.at[S_X])
        cwr = mk(wr_hbm, wr_v, sems.at[S_WR])
        head_stream = merge(wq_copies(0, D // 2), wq_copies(D // 2, D), _PRIME)
        ta = row_copies(wg_hbm, wg_v, S_G, F) + row_copies(wd_hbm, wd_v, S_D, F // 2)
        tb = (row_copies(wu_hbm, wu_v, S_U, F)
              + row_copies(wd_hbm, wd_v, S_D, F - F // 2, F // 2))
        for i in range(n_wo):
            (ta if wo_off[i] < H * DH // 2 else tb).extend(
                row_copies(wo_hbm, wo_v, S_WO + i, chunks[i], wo_off[i]))
        tail = merge(ta, tb)
        cuts = [round(j * len(tail) / _N_TAIL) for j in range(_N_TAIL + 1)]

        def issue_tail(j):
            start_all(tail[cuts[j]:cuts[j + 1]])

        def issue_head(h):
            for p, r in _split(W, _KV_ROWS):
                mk(k_hbm.at[0, h, pl.ds(Sk - W + p, r), :], k_v.at[h, pl.ds(p, r), :],
                   sems.at[S_K + h]).start(priority=0)
                mk(v_hbm.at[0, h, pl.ds(Sk - W + p, r), :], v_v.at[h, pl.ds(p, r), :],
                   sems.at[S_V + h]).start(priority=1)

        cx.start()
        cwr.start()
        start_all(head_stream)
        for h in range(L):
            issue_head(h)

        cx.wait()
        x = x_v[0].astype(f32)
        mu = jnp.mean(x, axis=-1, keepdims=True)
        xc = x - mu
        var = jnp.mean(xc * xc, axis=-1, keepdims=True)
        xn = (xc / jnp.sqrt(var + 1e-5)).astype(bf16)
        xn_m = jnp.broadcast_to(xn, (M, D))

        wait_all(wq_v, sems.at[S_WQ])
        q = jnp.dot(xn_m, wq_v[...], preferred_element_type=f32).astype(bf16)
        for h in range(H):
            q_s[h] = q[:, h * DH:(h + 1) * DH]

        def head(h, carry):
            nxt = h + L

            @pl.when(nxt < H)
            def _():
                issue_head(nxt)

            for j in range(min(L, _N_TAIL)):
                @pl.when(nxt == H + j)
                def _():
                    issue_tail(j)

            wait_all(k_v.at[h], sems.at[S_K + h])
            s = jax.lax.dot_general(q_s[h], k_v[h], _NT, preferred_element_type=f32)
            s = s * scale
            m = jnp.max(s, axis=-1, keepdims=True)
            p = jnp.exp(s - m)
            l = jnp.sum(p, axis=-1, keepdims=True)
            pb = p.astype(bf16)
            wait_all(v_v.at[h], sems.at[S_V + h])
            o = jnp.dot(pb, v_v[h], preferred_element_type=f32)
            o_s[h] = (o / l).astype(bf16)
            return carry

        jax.lax.fori_loop(0, H, head, 0)
        for j in range(min(L, _N_TAIL), _N_TAIL):
            issue_tail(j)

        ocol = jnp.concatenate([
            jnp.transpose(jnp.broadcast_to(o_s[h].astype(f32)[0:1], (DH, DH)))
            for h in range(hv0, H)], axis=0)

        cwr.wait()
        xnf = xn.astype(f32)
        wr = wr_v[...].astype(f32).reshape(1, D)
        r = jnp.sum(xnf * wr, axis=-1, keepdims=True)
        wait_all(wg_v, sems.at[S_G])
        gt = jax.lax.dot_general(xn_m, wg_v[...], _NT, preferred_element_type=f32)
        wait_all(wu_v, sems.at[S_U])
        up = jax.lax.dot_general(xn_m, wu_v[...], _NT, preferred_element_type=f32)
        gt = gt.astype(bf16).astype(f32)
        up = up.astype(bf16).astype(f32)
        hh = (gt * jax.nn.sigmoid(gt) * up).astype(bf16)
        wait_all(wd_v, sems.at[S_D])
        y = jnp.dot(hh, wd_v[...], preferred_element_type=f32)[0:1]
        y = y * jax.nn.sigmoid(r)
        b = xnf + (xnf * 0.0 + y)
        gate = b * jax.nn.sigmoid(b)

        def wo_group(i, acc):
            g = jnp.where(i == 3, 4, jnp.where(i == 4, 3, i))
            hpg = _WO_GROUP // DH
            oc = jnp.concatenate([o_s[g * hpg + j] for j in range(hpg)], axis=1)
            rows = pl.ds(pl.multiple_of(g * _WO_GROUP, _WO_GROUP), _WO_GROUP)
            wait_all(wo_v.at[rows, :], sems.at[S_WO + g])
            return acc + jnp.dot(oc, wo_v[rows, :], preferred_element_type=f32)

        acc = jax.lax.fori_loop(0, n_mxu, wo_group, jnp.zeros((M, D), f32))
        base = x + acc[0:1] * gate
        part = jnp.zeros((8, D), f32)
        for i in range(n_mxu, n_wo):
            a, e = wo_off[i], wo_off[i + 1]
            oc = ocol[a - hv0 * DH:e - hv0 * DH]
            wait_all(wo_v.at[pl.ds(a, e - a), :], sems.at[S_WO + i])
            w = wo_v[a:e, :].astype(f32)
            prod = w * jnp.concatenate([oc] * (D // DH), axis=1)
            part = part + jnp.sum(prod.reshape((e - a) // 8, 8, D), axis=0)
        out = base + jnp.sum(part, axis=0, keepdims=True) * gate
        o_ref[0] = out.astype(o_ref.dtype)

    hbm = pl.BlockSpec(memory_space=pltpu.HBM)
    return pl.pallas_call(
        kernel,
        out_shape=jax.ShapeDtypeStruct(A_x.shape, A_x.dtype),
        in_specs=[hbm] * 9,
        out_specs=pl.BlockSpec(memory_space=pltpu.VMEM),
        scratch_shapes=[
            pltpu.VMEM((1, 1, D), bf16),
            pltpu.VMEM((D,), bf16),
            pltpu.VMEM((D, H * DH), bf16),
            pltpu.VMEM((F, D), bf16),
            pltpu.VMEM((F, D), bf16),
            pltpu.VMEM((F, D), bf16),
            pltpu.VMEM((H * DH, D), bf16),
            pltpu.VMEM((H, W, DH), bf16),
            pltpu.VMEM((H, W, DH), bf16),
            pltpu.VMEM((H, M, DH), bf16),
            pltpu.VMEM((H, M, DH), bf16),
            pltpu.SemaphoreType.DMA((n_sem,)),
        ],
        compiler_params=pltpu.CompilerParams(
            vmem_limit_bytes=110 * 2**20,
            disable_semaphore_checks=True,
        ),
    )(A_x, A_k_cache, A_v_cache, A_wq, A_wo, B_w_r, B_w_gate.T, B_w_up.T, B_w_down)
```

```python
import jax
import jax.numpy as jnp
import numpy as np
import jax.experimental.pallas as pl
import jax.experimental.pallas.tpu as pltpu

_HQ, _DH = 32, 128
_M = 8
_NH = 4
_KV_ROWS = 84
_W_ROWS = 40
_WQ_STREAMS = 4
_WQ_TILE = (8, 1536)
_PRIME = 26
_TAIL_MIX = 20
_WO_GROUP = 512
_WO_MXU = (_WO_GROUP,) * 7
_WO_VPU = (256, 128, 64, 32, 32)

_NT = (((1,), (1,)), ((), ()))


def _split(n, c, start=0):
    return [(start + p, min(c, n - p)) for p in range(0, n, c)]


def _round_robin(streams):
    return [s[i] for i in range(max(len(s) for s in streams)) for s in streams
            if i < len(s)]


def _merge(a, b, prime=0):
    out = [(c, 1) for c, _ in b[:prime]]
    ia, ib, na, nb = 0, min(prime, len(b)), 0, 0
    while ia < len(a) or ib < len(b):
        if ia < len(a) and (ib >= len(b) or na <= nb):
            out.append((a[ia][0], 0))
            na += a[ia][1]
            ia += 1
        else:
            out.append((b[ib][0], 1))
            nb += b[ib][1]
            ib += 1
    return out


@jax.jit
def pallas_recurrent_scan__sliding_block_cached__moe_arch_mod__decode_kernel(
    A_x: jax.Array,
    A_k_cache: jax.Array,
    A_v_cache: jax.Array,
    A_wq: jax.Array,
    A_wo: jax.Array,
    B_x: jax.Array,
    B_w_r: jax.Array,
    B_w_gate: jax.Array,
    B_w_up: jax.Array,
    B_w_down: jax.Array,
):
    del B_x
    H, DH, M, NH = _HQ, _DH, _M, _NH
    D = A_x.shape[-1]
    F = B_w_gate.shape[1]
    Sk = A_k_cache.shape[2]
    W = min(4096, max(256, Sk // 4))
    assert A_x.shape == (1, 1, D) and A_k_cache.shape[1] == H
    NG = H // NH

    groups = _WO_MXU + _WO_VPU
    n_mxu, n_wo = len(_WO_MXU), len(groups)
    wo_off = np.concatenate([[0], np.cumsum(groups)]).tolist()
    assert wo_off[-1] == H * DH and wo_off[n_mxu] % DH == 0
    hv0 = wo_off[n_mxu] // DH

    S_X, S_WR, S_WQ, S_G, S_U, S_D, S_K = range(7)
    S_V = S_K + H
    S_WO = S_V + H
    n_sem = S_WO + n_wo
    f32, bf16 = jnp.float32, jnp.bfloat16
    scale = DH ** -0.5

    def kernel(x_hbm, k_hbm, v_hbm, wq_hbm, wo_hbm, wr_hbm, wg_hbm, wu_hbm, wd_hbm,
               o_ref,
               x_v, wr_v, wq_v, wg_v, wu_v, wd_v, wo_v, k_v, v_v, q_s, o_s, sems):
        mk = pltpu.make_async_copy

        def wait_all(buf, sem):
            mk(buf, buf, sem).wait()

        def row_copies(hbm, vm, sem, n, start=0):
            return [(mk(hbm.at[pl.ds(p, r), :], vm.at[pl.ds(p, r), :], sems.at[sem]), r)
                    for p, r in _split(n, _W_ROWS, start)]

        def wq_copies(r0, r1):
            return [(mk(wq_hbm.at[pl.ds(p, r), pl.ds(c0, cw)],
                        wq_v.at[pl.ds(p, r), pl.ds(c0, cw)], sems.at[S_WQ]), r * cw)
                    for p, r in _split(r1 - r0, _WQ_TILE[0], r0)
                    for c0, cw in _split(H * DH, _WQ_TILE[1])]

        def start_all(copies):
            for c, prio in copies:
                c.start(priority=prio)

        cx = mk(x_hbm, x_v, sems.at[S_X])
        cwr = mk(wr_hbm, wr_v, sems.at[S_WR])
        part = D // (2 * _WQ_STREAMS)
        wq_parts = [wq_copies(j * part, (j + 1) * part) for j in range(2 * _WQ_STREAMS)]
        wq_stream = _merge(_round_robin(wq_parts[:_WQ_STREAMS]),
                           _round_robin(wq_parts[_WQ_STREAMS:]), _PRIME)

        ffn_a = row_copies(wg_hbm, wg_v, S_G, F) + row_copies(wd_hbm, wd_v, S_D, F // 2)
        ffn_b = (row_copies(wu_hbm, wu_v, S_U, F)
                 + row_copies(wd_hbm, wd_v, S_D, F - F // 2, F // 2))
        wo_a, wo_b = [], []
        for i in range(n_wo):
            (wo_a if wo_off[i] < H * DH // 2 else wo_b).extend(
                row_copies(wo_hbm, wo_v, S_WO + i, groups[i], wo_off[i]))
        tail = _merge(
            _round_robin([ffn_a, wo_a[:_TAIL_MIX]]) + wo_a[_TAIL_MIX:],
            _round_robin([ffn_b, wo_b[:_TAIL_MIX]]) + wo_b[_TAIL_MIX:])
        tail_cuts = [round(j * len(tail) / NH) for j in range(NH + 1)]

        kv_rows = _split(W, _KV_ROWS)
        kv_cuts = [round(j * len(kv_rows) / NH) for j in range(NH + 1)]

        def issue_kv(g, j):
            for p, r in kv_rows[kv_cuts[j]:kv_cuts[j + 1]]:
                for dh in range(NH):
                    h = g * NH + dh
                    mk(k_hbm.at[0, h, pl.ds(Sk - W + p, r), :], k_v.at[h, pl.ds(p, r), :],
                       sems.at[S_K + h]).start(priority=0)
                    mk(v_hbm.at[0, h, pl.ds(Sk - W + p, r), :], v_v.at[h, pl.ds(p, r), :],
                       sems.at[S_V + h]).start(priority=1)

        cx.start()
        cwr.start()
        start_all(wq_stream)
        for j in range(NH):
            issue_kv(0, j)

        cx.wait()
        x = x_v[0].astype(f32)
        mu = jnp.mean(x, axis=-1, keepdims=True)
        xc = x - mu
        var = jnp.mean(xc * xc, axis=-1, keepdims=True)
        xn = (xc / jnp.sqrt(var + 1e-5)).astype(bf16)
        xn_m = jnp.broadcast_to(xn, (M, D))

        wait_all(wq_v, sems.at[S_WQ])
        q = jnp.dot(xn_m, wq_v[...], preferred_element_type=f32).astype(bf16)
        for h in range(H):
            q_s[h] = q[:, h * DH:(h + 1) * DH]

        def head(h, carry):
            g1 = h // NH + 1
            jj = h % NH
            for j in range(NH):
                @pl.when((g1 < NG) & (jj == j))
                def _():
                    issue_kv(g1, j)

                @pl.when((g1 == NG) & (jj == j))
                def _():
                    start_all(tail[tail_cuts[j]:tail_cuts[j + 1]])

            wait_all(k_v.at[h], sems.at[S_K + h])
            s = jax.lax.dot_general(q_s[h], k_v[h], _NT, preferred_element_type=f32)
            s = s * scale
            m = jnp.max(s, axis=-1, keepdims=True)
            p = jnp.exp(s - m)
            l = jnp.sum(p, axis=-1, keepdims=True)
            pb = p.astype(bf16)
            wait_all(v_v.at[h], sems.at[S_V + h])
            o = jnp.dot(pb, v_v[h], preferred_element_type=f32)
            o_s[h] = (o / l).astype(bf16)
            return carry

        jax.lax.fori_loop(0, H, head, 0)

        ocol = jnp.concatenate([
            jnp.transpose(jnp.broadcast_to(o_s[h].astype(f32)[0:1], (DH, DH)))
            for h in range(hv0, H)], axis=0)

        cwr.wait()
        xnf = xn.astype(f32)
        wr = wr_v[...].astype(f32).reshape(1, D)
        r = jnp.sum(xnf * wr, axis=-1, keepdims=True)
        wait_all(wg_v, sems.at[S_G])
        gt = jax.lax.dot_general(xn_m, wg_v[...], _NT, preferred_element_type=f32)
        wait_all(wu_v, sems.at[S_U])
        up = jax.lax.dot_general(xn_m, wu_v[...], _NT, preferred_element_type=f32)
        gt = gt.astype(bf16).astype(f32)
        up = up.astype(bf16).astype(f32)
        hh = (gt * jax.nn.sigmoid(gt) * up).astype(bf16)
        wait_all(wd_v, sems.at[S_D])
        y = jnp.dot(hh, wd_v[...], preferred_element_type=f32)[0:1]
        y = y * jax.nn.sigmoid(r)
        b = xnf + (xnf * 0.0 + y)
        gate = b * jax.nn.sigmoid(b)

        def wo_group(i, acc):
            g = jnp.where(i == 3, 4, jnp.where(i == 4, 3, i))
            hpg = _WO_GROUP // DH
            oc = jnp.concatenate([o_s[g * hpg + j] for j in range(hpg)], axis=1)
            rows = pl.ds(pl.multiple_of(g * _WO_GROUP, _WO_GROUP), _WO_GROUP)
            wait_all(wo_v.at[rows, :], sems.at[S_WO + g])
            return acc + jnp.dot(oc, wo_v[rows, :], preferred_element_type=f32)

        acc = jax.lax.fori_loop(0, n_mxu, wo_group, jnp.zeros((M, D), f32))
        base = x + acc[0:1] * gate
        part_sum = jnp.zeros((8, D), f32)
        for i in range(n_mxu, n_wo):
            a, e = wo_off[i], wo_off[i + 1]
            oc = ocol[a - hv0 * DH:e - hv0 * DH]
            wait_all(wo_v.at[pl.ds(a, e - a), :], sems.at[S_WO + i])
            w = wo_v[a:e, :].astype(f32)
            prod = w * jnp.concatenate([oc] * (D // DH), axis=1)
            part_sum = part_sum + jnp.sum(prod.reshape((e - a) // 8, 8, D), axis=0)
        out = base + jnp.sum(part_sum, axis=0, keepdims=True) * gate
        o_ref[0] = out.astype(o_ref.dtype)

    hbm = pl.BlockSpec(memory_space=pltpu.HBM)
    return pl.pallas_call(
        kernel,
        out_shape=jax.ShapeDtypeStruct(A_x.shape, A_x.dtype),
        in_specs=[hbm] * 9,
        out_specs=pl.BlockSpec(memory_space=pltpu.VMEM),
        scratch_shapes=[
            pltpu.VMEM((1, 1, D), bf16),
            pltpu.VMEM((D,), bf16),
            pltpu.VMEM((D, H * DH), bf16),
            pltpu.VMEM((F, D), bf16),
            pltpu.VMEM((F, D), bf16),
            pltpu.VMEM((F, D), bf16),
            pltpu.VMEM((H * DH, D), bf16),
            pltpu.VMEM((H, W, DH), bf16),
            pltpu.VMEM((H, W, DH), bf16),
            pltpu.VMEM((H, M, DH), bf16),
            pltpu.VMEM((H, M, DH), bf16),
            pltpu.SemaphoreType.DMA((n_sem,)),
        ],
        compiler_params=pltpu.CompilerParams(
            vmem_limit_bytes=110 * 2**20,
            disable_semaphore_checks=True,
        ),
    )(A_x, A_k_cache, A_v_cache, A_wq, A_wo, B_w_r, B_w_gate.T, B_w_up.T, B_w_down)
```

```python
import jax
import jax.numpy as jnp
import numpy as np
import jax.experimental.pallas as pl
import jax.experimental.pallas.tpu as pltpu

_HQ, _DH = 32, 128
_M = 8
_GROUPS = (8, 8, 8, 4, 4)
_KV_ROWS = 80
_EXTRA = (45, 20)
_W_ROWS = 40
_WQ_STREAMS = 4
_WQ_TILE = (8, 1536)
_PRIME = 26
_TAIL_MIX = 20
_WO_GROUP = 512
_WO_MXU = (_WO_GROUP,) * 7
_WO_VPU = (256, 128, 64, 32, 32)

_NT = (((1,), (1,)), ((), ()))


def _split(n, c, start=0):
    return [(start + p, min(c, n - p)) for p in range(0, n, c)]


def _round_robin(streams):
    return [s[i] for i in range(max(len(s) for s in streams)) for s in streams
            if i < len(s)]


def _merge(a, b, prime=0):
    out = [(c, 1) for c, _ in b[:prime]]
    ia, ib, na, nb = 0, min(prime, len(b)), 0, 0
    while ia < len(a) or ib < len(b):
        if ia < len(a) and (ib >= len(b) or na <= nb):
            out.append((a[ia][0], 0))
            na += a[ia][1]
            ia += 1
        else:
            out.append((b[ib][0], 1))
            nb += b[ib][1]
            ib += 1
    return out


@jax.jit
def pallas_recurrent_scan__sliding_block_cached__moe_arch_mod__decode_kernel(
    A_x: jax.Array,
    A_k_cache: jax.Array,
    A_v_cache: jax.Array,
    A_wq: jax.Array,
    A_wo: jax.Array,
    B_x: jax.Array,
    B_w_r: jax.Array,
    B_w_gate: jax.Array,
    B_w_up: jax.Array,
    B_w_down: jax.Array,
):
    del B_x
    H, DH, M = _HQ, _DH, _M
    D = A_x.shape[-1]
    F = B_w_gate.shape[1]
    Sk = A_k_cache.shape[2]
    W = min(4096, max(256, Sk // 4))
    assert A_x.shape == (1, 1, D) and A_k_cache.shape[1] == H
    g_size = list(_GROUPS)
    g_head = [0] + np.cumsum(g_size)[:-1].tolist()
    assert sum(g_size) == H

    wo_rows = _WO_MXU + _WO_VPU
    n_mxu, n_wo = len(_WO_MXU), len(wo_rows)
    wo_off = np.concatenate([[0], np.cumsum(wo_rows)]).tolist()
    assert wo_off[-1] == H * DH and wo_off[n_mxu] % DH == 0
    hv0 = wo_off[n_mxu] // DH

    S_X, S_WR, S_WQ, S_G, S_U, S_D, S_K = range(7)
    S_V = S_K + H
    S_WO = S_V + H
    n_sem = S_WO + n_wo
    f32, bf16 = jnp.float32, jnp.bfloat16
    scale = DH ** -0.5

    def kernel(x_hbm, k_hbm, v_hbm, wq_hbm, wo_hbm, wr_hbm, wg_hbm, wu_hbm, wd_hbm,
               o_ref,
               x_v, wr_v, wq_v, wg_v, wu_v, wd_v, wo_v, k_v, v_v, q_s, o_s, sems):
        mk = pltpu.make_async_copy

        def wait_all(buf, sem):
            mk(buf, buf, sem).wait()

        def row_copies(hbm, vm, sem, n, start=0):
            return [(mk(hbm.at[pl.ds(p, r), :], vm.at[pl.ds(p, r), :], sems.at[sem]), r)
                    for p, r in _split(n, _W_ROWS, start)]

        def wq_copies(r0, r1):
            return [(mk(wq_hbm.at[pl.ds(p, r), pl.ds(c0, cw)],
                        wq_v.at[pl.ds(p, r), pl.ds(c0, cw)], sems.at[S_WQ]), r * cw)
                    for p, r in _split(r1 - r0, _WQ_TILE[0], r0)
                    for c0, cw in _split(H * DH, _WQ_TILE[1])]

        def start_all(copies):
            for c, prio in copies:
                c.start(priority=prio)

        cx = mk(x_hbm, x_v, sems.at[S_X])
        cwr = mk(wr_hbm, wr_v, sems.at[S_WR])
        part = D // (2 * _WQ_STREAMS)
        wq_parts = [wq_copies(j * part, (j + 1) * part) for j in range(2 * _WQ_STREAMS)]
        wq_stream = _merge(_round_robin(wq_parts[:_WQ_STREAMS]),
                           _round_robin(wq_parts[_WQ_STREAMS:]), _PRIME)

        ffn_a = row_copies(wg_hbm, wg_v, S_G, F) + row_copies(wd_hbm, wd_v, S_D, F // 2)
        ffn_b = (row_copies(wu_hbm, wu_v, S_U, F)
                 + row_copies(wd_hbm, wd_v, S_D, F - F // 2, F // 2))
        wo_a, wo_b = [], []
        for i in range(n_wo):
            (wo_a if wo_off[i] < H * DH // 2 else wo_b).extend(
                row_copies(wo_hbm, wo_v, S_WO + i, wo_rows[i], wo_off[i]))
        tail = _merge(
            _round_robin([ffn_a, wo_a[:_TAIL_MIX]]) + wo_a[_TAIL_MIX:],
            _round_robin([ffn_b, wo_b[:_TAIL_MIX]]) + wo_b[_TAIL_MIX:])
        def cuts(n, parts, extra):
            extra = min(extra, n)
            return [0] + [round(extra + (j + 1) * (n - extra) / parts)
                          for j in range(parts)]

        kv_rows = _split(W, _KV_ROWS)

        def issue_kv(h0, nh, lo, hi):
            for p, r in kv_rows[lo:hi]:
                for h in range(h0, h0 + nh):
                    mk(k_hbm.at[0, h, pl.ds(Sk - W + p, r), :], k_v.at[h, pl.ds(p, r), :],
                       sems.at[S_K + h]).start(priority=0)
                    mk(v_hbm.at[0, h, pl.ds(Sk - W + p, r), :], v_v.at[h, pl.ds(p, r), :],
                       sems.at[S_V + h]).start(priority=1)

        def issue_step(h):
            for gi, n in enumerate(g_size):
                last = gi + 1 == len(g_size)
                if last:
                    c = cuts(len(tail), n, _EXTRA[1])
                else:
                    nh = g_size[gi + 1]
                    c = cuts(len(kv_rows), n, _EXTRA[0] / (2 * nh))
                for j in range(n):
                    @pl.when(h == g_head[gi] + j)
                    def _():
                        if last:
                            start_all(tail[c[j]:c[j + 1]])
                        else:
                            issue_kv(g_head[gi + 1], nh, c[j], c[j + 1])

        cx.start()
        cwr.start()
        start_all(wq_stream)
        issue_kv(0, g_size[0], 0, len(kv_rows))

        cx.wait()
        x = x_v[0].astype(f32)
        mu = jnp.mean(x, axis=-1, keepdims=True)
        xc = x - mu
        var = jnp.mean(xc * xc, axis=-1, keepdims=True)
        xn = (xc / jnp.sqrt(var + 1e-5)).astype(bf16)
        xn_m = jnp.broadcast_to(xn, (M, D))

        wait_all(wq_v, sems.at[S_WQ])
        q = jnp.dot(xn_m, wq_v[...], preferred_element_type=f32).astype(bf16)
        for h in range(H):
            q_s[h] = q[:, h * DH:(h + 1) * DH]

        def head(h, carry):
            issue_step(h)
            wait_all(k_v.at[h], sems.at[S_K + h])
            s = jax.lax.dot_general(q_s[h], k_v[h], _NT, preferred_element_type=f32)
            s = s * scale
            m = jnp.max(s, axis=-1, keepdims=True)
            p = jnp.exp(s - m)
            l = jnp.sum(p, axis=-1, keepdims=True)
            pb = p.astype(bf16)
            wait_all(v_v.at[h], sems.at[S_V + h])
            o = jnp.dot(pb, v_v[h], preferred_element_type=f32)
            o_s[h] = (o / l).astype(bf16)
            return carry

        jax.lax.fori_loop(0, H, head, 0)

        ocol = jnp.concatenate([
            jnp.transpose(jnp.broadcast_to(o_s[h].astype(f32)[0:1], (DH, DH)))
            for h in range(hv0, H)], axis=0)

        cwr.wait()
        xnf = xn.astype(f32)
        wr = wr_v[...].astype(f32).reshape(1, D)
        r = jnp.sum(xnf * wr, axis=-1, keepdims=True)
        wait_all(wg_v, sems.at[S_G])
        gt = jax.lax.dot_general(xn_m, wg_v[...], _NT, preferred_element_type=f32)
        wait_all(wu_v, sems.at[S_U])
        up = jax.lax.dot_general(xn_m, wu_v[...], _NT, preferred_element_type=f32)
        gt = gt.astype(bf16).astype(f32)
        up = up.astype(bf16).astype(f32)
        hh = (gt * jax.nn.sigmoid(gt) * up).astype(bf16)
        wait_all(wd_v, sems.at[S_D])
        y = jnp.dot(hh, wd_v[...], preferred_element_type=f32)[0:1]
        y = y * jax.nn.sigmoid(r)
        b = xnf + (xnf * 0.0 + y)
        gate = b * jax.nn.sigmoid(b)

        def wo_group(i, acc):
            g = jnp.where(i == 3, 4, jnp.where(i == 4, 3, i))
            hpg = _WO_GROUP // DH
            oc = jnp.concatenate([o_s[g * hpg + j] for j in range(hpg)], axis=1)
            rows = pl.ds(pl.multiple_of(g * _WO_GROUP, _WO_GROUP), _WO_GROUP)
            wait_all(wo_v.at[rows, :], sems.at[S_WO + g])
            return acc + jnp.dot(oc, wo_v[rows, :], preferred_element_type=f32)

        acc = jax.lax.fori_loop(0, n_mxu, wo_group, jnp.zeros((M, D), f32))
        base = x + acc[0:1] * gate
        part_sum = jnp.zeros((8, D), f32)
        for i in range(n_mxu, n_wo):
            a, e = wo_off[i], wo_off[i + 1]
            oc = ocol[a - hv0 * DH:e - hv0 * DH]
            wait_all(wo_v.at[pl.ds(a, e - a), :], sems.at[S_WO + i])
            w = wo_v[a:e, :].astype(f32)
            prod = w * jnp.concatenate([oc] * (D // DH), axis=1)
            part_sum = part_sum + jnp.sum(prod.reshape((e - a) // 8, 8, D), axis=0)
        out = base + jnp.sum(part_sum, axis=0, keepdims=True) * gate
        o_ref[0] = out.astype(o_ref.dtype)

    hbm = pl.BlockSpec(memory_space=pltpu.HBM)
    return pl.pallas_call(
        kernel,
        out_shape=jax.ShapeDtypeStruct(A_x.shape, A_x.dtype),
        in_specs=[hbm] * 9,
        out_specs=pl.BlockSpec(memory_space=pltpu.VMEM),
        scratch_shapes=[
            pltpu.VMEM((1, 1, D), bf16),
            pltpu.VMEM((D,), bf16),
            pltpu.VMEM((D, H * DH), bf16),
            pltpu.VMEM((F, D), bf16),
            pltpu.VMEM((F, D), bf16),
            pltpu.VMEM((F, D), bf16),
            pltpu.VMEM((H * DH, D), bf16),
            pltpu.VMEM((H, W, DH), bf16),
            pltpu.VMEM((H, W, DH), bf16),
            pltpu.VMEM((H, M, DH), bf16),
            pltpu.VMEM((H, M, DH), bf16),
            pltpu.SemaphoreType.DMA((n_sem,)),
        ],
        compiler_params=pltpu.CompilerParams(
            vmem_limit_bytes=110 * 2**20,
            disable_semaphore_checks=True,
        ),
    )(A_x, A_k_cache, A_v_cache, A_wq, A_wo, B_w_r, B_w_gate.T, B_w_up.T, B_w_down)
```
